```python
import jax
import jax.numpy as jnp

def _softmax(x, axis=-1):
    return jax.nn.softmax(x, axis=axis)

def _gelu(x):
    return jax.nn.gelu(x, approximate=True)

def _silu(x):
    return jax.nn.silu(x)

def _sigmoid(x):
    return jax.nn.sigmoid(x)

def _layernorm(x, axis=-1, eps=1e-05):
    m = jnp.mean(x, axis=axis, keepdims=True)
    v = jnp.var(x, axis=axis, keepdims=True)
    return (x - m) / jnp.sqrt(v + eps)

def _scatter_add(tgt, idx, src, axis=0):
    return tgt.at[idx].add(src)

def _segment_sum(src, seg, n):
    return jax.ops.segment_sum(src, seg, n)

class _Rng:

    def __init__(self, key):
        self._k = key

    def _next(self):
        self._k, sub = jax.random.split(self._k)
        return sub

    def normal(self, shape):
        return jax.random.normal(self._next(), shape, dtype=jnp.bfloat16)

    def randint(self, lo, hi, shape):
        return jax.random.randint(self._next(), shape, lo, hi, dtype=jnp.int32)

    def uniform(self, shape, lo=0.0, hi=1.0):
        return jax.random.uniform(self._next(), shape, jnp.bfloat16, lo, hi)

    def permutation(self, n):
        return jax.random.permutation(self._next(), n)
kernel_name = 'adaLN_cond__grouped_kv_mqa__mixer_token_mlp__prompt'

def _fwd_setup_inputs():
    _rng = _Rng(jax.random.key(int.from_bytes(__import__("os").urandom(4), "little")))
    _w = lambda a: (lambda t: t.astype(jnp.bfloat16) if jnp.issubdtype(t.dtype, jnp.floating) else t)(jnp.asarray(a))

    def _A_setup():
        B, S, D, H = (1, 2048, 512, 32)
        Dh = D // H
        return {'x': _w((lambda *s: _rng.normal(s) * 0.05)(B, S, D)), 'wq': _w((lambda *s: _rng.normal(s) * 0.05)(D, H * Dh)), 'wk': _w((lambda *s: _rng.normal(s) * 0.05)(D, Dh)), 'wv': _w((lambda *s: _rng.normal(s) * 0.05)(D, Dh)), 'wo': _w((lambda *s: _rng.normal(s) * 0.05)(H * Dh, D))}
    _A_in = _A_setup()

    def _B_setup():
        B, S, D, F = (1, 2048, 512, 1376)
        return {'x': _w((lambda *s: _rng.normal(s) * 0.05)(B, S, D)), 'w1': _w((lambda *s: _rng.normal(s) * 0.05)(S, F) * S ** (-0.5)), 'b1': _w((lambda *s: _rng.normal(s) * 0.05)(F) * 0.02), 'w2': _w((lambda *s: _rng.normal(s) * 0.05)(F, S) * F ** (-0.5)), 'b2': _w((lambda *s: _rng.normal(s) * 0.05)(S) * 0.02)}
    _B_in = _B_setup()
    return {'A_x': _A_in['x'], 'A_wq': _A_in['wq'], 'A_wk': _A_in['wk'], 'A_wv': _A_in['wv'], 'A_wo': _A_in['wo'], 'B_x': _B_in['x'], 'B_w1': _B_in['w1'], 'B_b1': _B_in['b1'], 'B_w2': _B_in['w2'], 'B_b2': _B_in['b2'], 'c': _w((lambda *s: _rng.normal(s) * 0.05)(1, 512)), 'w_mod': _w((lambda *s: _rng.normal(s) * 0.05)(512, 6 * 512) * 512 ** (-0.5))}

def _fwd_reference(A_x, A_wq, A_wk, A_wv, A_wo, B_x, B_w1, B_b1, B_w2, B_b2, c, w_mod):

    def _A_ref(x, wq, wk, wv, wo):
        B, S, D = x.shape
        H = 32
        Dh = D // H
        q = (lambda x, *d: x.transpose(*d))((x @ wq).reshape(B, S, H, Dh), 0, 2, 1, 3)
        k = x @ wk
        v = x @ wv
        scores = jnp.einsum('bhqd,bkd->bhqk', q, k) * Dh ** (-0.5)
        p = _softmax(scores, axis=-1)
        o = jnp.einsum('bhqk,bkd->bhqd', p, v)
        return (lambda x, *d: x.transpose(*d))(o, 0, 2, 1, 3).reshape(B, S, H * Dh) @ wo

    def _B_ref(x, w1, b1, w2, b2):
        B, S, D = x.shape
        h = _layernorm(x, axis=-1)
        u = jnp.einsum('bsd,sf->bdf', h, w1) + b1
        u = _gelu(u)
        y = jnp.einsum('bdf,fs->bds', u, w2) + b2
        return (lambda x, *d: x.transpose(*d))(y, 0, 2, 1)
    x = A_x
    mod = (_silu(c) @ w_mod).reshape(c.shape[0], 6, 1, -1)
    sa, ca, ga, sb, cb, gb = (mod[:, 0].copy(), mod[:, 1].copy(), mod[:, 2].copy(), mod[:, 3].copy(), mod[:, 4].copy(), mod[:, 5].copy())
    h = _layernorm(x, axis=-1) * (1 + ca) + sa
    x = x + ga * _A_ref(h, A_wq, A_wk, A_wv, A_wo)
    h = _layernorm(x, axis=-1) * (1 + cb) + sb
    x = x + gb * _B_ref(h, B_w1, B_b1, B_w2, B_b2)
    return x

def setup_inputs():
    _inp = _fwd_setup_inputs()
    _gk = jax.random.fold_in(jax.random.key(int.from_bytes(__import__("os").urandom(4), "little")), 2 ** 31 - 1)
    _shapes = [[1, 2048, 512]]
    _dtypes = ['bfloat16']
    _gks = jax.random.split(_gk, len(_shapes))
    _gs = [jax.random.normal(k, s, dtype=jnp.dtype(d)) * 0.05 for k, s, d in zip(_gks, _shapes, _dtypes)]
    _inp['grad_out'] = _gs[0]
    return _inp

def reference(A_x, A_wq, A_wk, A_wv, A_wo, B_w1, B_b1, B_w2, B_b2, c, w_mod, B_x, grad_out):
    _const = dict(B_x=B_x)

    def _f(*_d):
        return _fwd_reference(**{'A_x': _d[0], 'A_wq': _d[1], 'A_wk': _d[2], 'A_wv': _d[3], 'A_wo': _d[4], 'B_w1': _d[5], 'B_b1': _d[6], 'B_w2': _d[7], 'B_b2': _d[8], 'c': _d[9], 'w_mod': _d[10], **_const})
    _out, _vjp = jax.vjp(_f, A_x, A_wq, A_wk, A_wv, A_wo, B_w1, B_b1, B_w2, B_b2, c, w_mod)
    _grads = _vjp(grad_out)
    _out0 = jnp.asarray(_out)
    return (_out0, *[jnp.asarray(_g) for _g in _grads])
```

```python
import math

import jax
import jax.numpy as jnp
from jax import lax
import jax.experimental.pallas as pl
import jax.experimental.pallas.tpu as pltpu

F32 = jnp.float32
BF16 = jnp.bfloat16
U32 = jnp.uint32

S = 2048
D = 512
H = 32
DH = 16
F = 1376
EPS = 1e-5
LOG2E = math.log2(math.e)
SCALE = DH ** -0.5

KT = 128
NKT = S // KT
CW = 512
UN = 2
BQ = CW * UN
NQ = S // BQ
NB = H * NQ
N_HBM = 31
N_VMEM = 17
N_REC = NB - N_HBM - N_VMEM
LAG = 2

TC = 512
NTC = S // TC
FC = 256
NFC = F // FC
FTAIL = F - NFC * FC
FPAD = -(-F // 128) * 128

NT_DIMS = (((1,), (1,)), ((), ()))


def _dot(a, b):
    return jnp.dot(a, b, preferred_element_type=F32)


def _dot_nt(a, b):
    return lax.dot_general(a, b, NT_DIMS, preferred_element_type=F32)


def _lanes(col, n):
    return jnp.concatenate([col] * (n // 128), axis=1)


def _fold_lanes(x):
    acc = x[:, 0:128]
    for j in range(1, x.shape[1] // 128):
        acc = acc + x[:, j * 128:(j + 1) * 128]
    return acc


def _row_to_col(row):
    n = row.shape[1]
    return jnp.concatenate(
        [jnp.broadcast_to(row[:, j:j + 128], (128, 128)).T for j in range(0, n, 128)], axis=0)


def _col_sum_to_row(part):
    return jnp.sum(part.T, axis=0, keepdims=True)


def _ln(x):
    xc = x - jnp.mean(x, axis=0, keepdims=True)
    rstd = lax.rsqrt(jnp.mean(xc * xc, axis=0, keepdims=True) + EPS)
    return xc * rstd, rstd


def _ln_bwd(dy, xhat, rstd):
    return rstd * (dy - jnp.mean(dy, axis=0, keepdims=True)
                   - xhat * jnp.mean(dy * xhat, axis=0, keepdims=True))


def _gelu_and_grad(u):
    k0 = math.sqrt(2.0 / math.pi)
    k1 = 0.044715
    u2 = u * u
    t = jnp.tanh(u * (k0 + (k0 * k1) * u2))
    cdf = 0.5 + 0.5 * t
    grad = cdf + (0.5 * u) * (1.0 - t * t) * (k0 + (3.0 * k0 * k1) * u2)
    return u * cdf, grad


def _kernel(
    c_ref, b1_ref, b2_ref, wkT_ref, wvT_ref,
    x_hbm, go_hbm, wq_hbm, wo_hbm, w1T_hbm, w2_hbm, wm_hbm,
    dwkT_ref, dwvT_ref, db1_ref, db2_ref, dc_ref,
    out_hbm, dx_hbm, dwq_hbm, dwo_hbm, dw1T_hbm, dw2_hbm, dwm_hbm, p_hbm,
    p_scr, xT_scr, qT_scr, oT_scr, k_scr, v_scr, kT_scr, vT_scr, m_scr, linv_scr, delta_scr,
    a1_scr, a0_scr, dcp_scr, p_sems, sems,
):
    c = c_ref[...].astype(F32)
    sig_c = jax.nn.sigmoid(c)
    sc = (c * sig_c).astype(BF16)
    sc16 = jnp.broadcast_to(sc, (16, D))

    def qslice(b, u):
        h = lax.shift_right_logical(b, NQ.bit_length() - 1)
        j = b & (NQ - 1)
        cols = pl.ds(pl.multiple_of(j * BQ + u * CW, CW), CW)
        return h, pl.ds(pl.multiple_of(h * DH, DH), DH), cols

    def key_rows(ref, kt):
        return pltpu.bitcast(ref[pl.ds(kt * (KT // 2), KT // 2), :], BF16)

    def key_cols(ref, kt):
        return pltpu.bitcast(ref[:, pl.ds(kt * KT, KT)], BF16)

    def phase_qkv(x_buf, wm_buf, wq_buf, wT_scr):
        wm_cp = pltpu.make_async_copy(wm_hbm.at[:, pl.ds(0, 2 * D)], wm_buf, sems.at[0])
        wq_cp = pltpu.make_async_copy(wq_hbm, wq_buf, sems.at[1])
        x_cps = [
            pltpu.make_async_copy(x_hbm.at[pl.ds(t * TC, TC)], x_buf.at[t], sems.at[2 + t])
            for t in range(NTC)
        ]
        wm_cp.start()
        x_cps[0].start()
        wq_cp.start()
        for cp in x_cps[1:]:
            cp.start()
        wm_cp.wait()
        mod = _dot(sc16, wm_buf[...])[0:1]
        a0_scr[...] = _row_to_col(mod[:, 0:D])
        a1_scr[...] = _row_to_col(1.0 + mod[:, D:2 * D])
        wq_cp.wait()
        wT_scr[0:D, :] = wq_buf[...].T
        wT_scr[D:D + DH, :] = wkT_ref[...]
        wT_scr[D + DH:D + 2 * DH, :] = wvT_ref[...]
        for t in range(NTC):
            cols = pl.ds(t * TC, TC)
            x_cps[t].wait()
            xT = x_buf[t].T
            xT_scr[:, cols] = xT
            xhat, _ = _ln(xT.astype(F32))
            hT = (xhat * _lanes(a1_scr[...], TC) + _lanes(a0_scr[...], TC)).astype(BF16)
            qkv = _dot(wT_scr[...], hT)
            qT_scr[:, cols] = (qkv[0:D] * (SCALE * LOG2E)).astype(BF16)
            kT = qkv[D:D + DH]
            vT = qkv[D + DH:D + 2 * DH]
            kT_scr[:, cols] = pltpu.bitcast(kT.astype(BF16), U32)
            vT_scr[:, cols] = pltpu.bitcast(vT.astype(BF16), U32)
            rows = pl.ds(t * (TC // 2), TC // 2)
            k_scr[rows, :] = pltpu.bitcast(kT.T.astype(BF16), U32)
            v_scr[rows, :] = pltpu.bitcast(vT.T.astype(BF16), U32)

    with jax.named_scope("qkv"):
        pl.run_scoped(
            phase_qkv,
            pltpu.VMEM((NTC, TC, D), BF16), pltpu.VMEM((D, 2 * D), BF16), pltpu.VMEM((D, D), BF16),
            pltpu.VMEM((D + 2 * DH, D), BF16),
        )

    def spill(n):
        slot = lax.rem(n, N_VMEM)
        return pltpu.make_async_copy(p_scr.at[slot], p_hbm.at[n], p_sems.at[slot])

    def fill(n):
        slot = lax.rem(n, N_VMEM)
        return pltpu.make_async_copy(p_hbm.at[n], p_scr.at[slot], p_sems.at[slot])

    def phase_attn_fwd(s_scr, mcur_scr):
        for u in range(UN):
            q = qT_scr[0:DH, u * CW:(u + 1) * CW]
            mx = None
            for kt in range(NKT):
                s = _dot(key_rows(k_scr, kt), q)
                s_scr[u, pl.ds(kt * KT, KT), :] = s
                t = jnp.max(s.reshape(KT // 8, 8, CW), axis=0)
                mx = t if mx is None else jnp.maximum(mx, t)
            mcur_scr[u] = jnp.broadcast_to(jnp.max(mx, axis=0, keepdims=True), (8, CW))

        def step(b, with_next):
            n = jnp.where(b < N_HBM, b, jnp.maximum(b - N_REC, N_HBM))
            claims_slot = jnp.logical_or(b <= N_HBM, b > N_HBM + N_REC)
            slot = lax.rem(n, N_VMEM)

            @pl.when(jnp.logical_and(claims_slot, n >= N_VMEM))
            def _():
                spill(n - N_VMEM).wait()

            for u in range(UN):
                h, rows, cols = qslice(b, u)
                if with_next:
                    _, rows_n, cols_n = qslice(b + 1, u)
                    q_next = qT_scr[rows_n, cols_n]
                m = mcur_scr[u]
                mx = l = o = None
                for kt in range(NKT):
                    keys = pl.ds(kt * KT, KT)
                    p = jnp.exp2(s_scr[u, keys, :].reshape(KT // 8, 8, CW) - m[None])
                    for r in reversed(range(KT // 8)):
                        l = p[r] if l is None else l + p[r]
                    pb = p.reshape(KT, CW).astype(BF16)
                    p_scr[slot, u, pl.ds(kt * (KT // 2), KT // 2), :] = pltpu.bitcast(pb, U32)
                    t = _dot(key_cols(vT_scr, kt), pb)
                    o = t if o is None else o + t
                    if with_next:
                        s = _dot(key_rows(k_scr, kt), q_next)
                        s_scr[u, keys, :] = s
                        for r in range(KT // 8):
                            t = s[r * 8:(r + 1) * 8]
                            mx = t if mx is None else jnp.maximum(mx, t)
                linv = 1.0 / jnp.sum(l, axis=0, keepdims=True)
                oT_scr[rows, cols] = (o * linv).astype(BF16)
                linv_scr[pl.ds(h, 1), cols] = linv
                m_scr[pl.ds(h, 1), cols] = m[0:1]
                if with_next:
                    mcur_scr[u] = jnp.broadcast_to(jnp.max(mx, axis=0, keepdims=True), (8, CW))

            @pl.when(b < N_HBM)
            def _():
                spill(b).start()

        def body(b, carry):
            step(b, True)
            return carry

        lax.fori_loop(0, NB - 1, body, 0)
        step(jnp.int32(NB - 1), False)

    with jax.named_scope("attn_fwd"):
        pl.run_scoped(phase_attn_fwd, pltpu.VMEM((UN, S, CW), F32), pltpu.VMEM((UN, 8, CW), F32))

    def phase_rest(dx1_scr):
        def phase_mid(io_buf, goT_scr, hnT_scr, wo_buf, woT_scr, wm_buf, col_scr, b1c_scr, w1_buf,
                      w2_buf, dw1_buf, dw2_buf, y_scr, dhn_scr, db1_scr, g_scr, part_scr):
            x1T_scr = dx1_scr
            wo_cp = pltpu.make_async_copy(wo_hbm, wo_buf, sems.at[0])
            wm_cp = pltpu.make_async_copy(wm_hbm.at[:, pl.ds(2 * D, 4 * D)], wm_buf, sems.at[1])
            go_cps = [
                pltpu.make_async_copy(go_hbm.at[pl.ds(t * TC, TC)], io_buf.at[t], sems.at[2 + t])
                for t in range(NTC)
            ]

            def w_cps(f, slot, n):
                rows = pl.ds(pl.multiple_of(f * FC, FC), n)
                return (
                    pltpu.make_async_copy(w1T_hbm.at[rows], w1_buf.at[slot, pl.ds(0, n)], sems.at[6 + slot]),
                    pltpu.make_async_copy(w2_hbm.at[rows], w2_buf.at[slot, pl.ds(0, n)], sems.at[8 + slot]),
                )

            def dw_cps(f, slot, n):
                rows = pl.ds(pl.multiple_of(f * FC, FC), n)
                return (
                    pltpu.make_async_copy(dw1_buf.at[slot, pl.ds(0, n)], dw1T_hbm.at[rows], sems.at[10 + slot]),
                    pltpu.make_async_copy(dw2_buf.at[slot, pl.ds(0, n)], dw2_hbm.at[rows], sems.at[12 + slot]),
                )

            wo_cp.start()
            wm_cp.start()
            for cp in go_cps:
                cp.start()
            for cp in w_cps(NFC, NFC & 1, FTAIL):
                cp.start()
            for cp in w_cps(NFC - 1, (NFC - 1) & 1, FC):
                cp.start()

            b1 = b1_ref[...].astype(F32).reshape(1, F)
            b1 = jnp.concatenate([b1, jnp.zeros((1, FPAD - F), F32)], axis=1)
            b1c_scr[...] = _row_to_col(b1)
            b2 = b2_ref[...].astype(F32).reshape(1, S)
            wo_cp.wait()
            woT_scr[...] = wo_buf[...].T
            wm_cp.wait()
            mod = _dot(sc16, wm_buf[...])[0:1]
            ga, sb, cb, gb = (mod[:, i * D:(i + 1) * D] for i in range(4))
            col_scr[0] = _row_to_col(ga)
            col_scr[1] = _row_to_col(sb)
            col_scr[2] = _row_to_col(1.0 + cb)
            col_scr[3] = _row_to_col(gb)

            def two_ln(x1):
                xh1, rstd1 = _ln(x1)
                hn, rstd2 = _ln(xh1 * _lanes(col_scr[2], TC) + _lanes(col_scr[1], TC))
                return xh1, rstd1, hn, rstd2

            db2 = []
            for t in range(NTC):
                cols = pl.ds(t * TC, TC)
                aT = _dot(woT_scr[...], oT_scr[:, cols])
                x1 = (xT_scr[:, cols].astype(F32) + _lanes(col_scr[0], TC) * aT).astype(BF16)
                x1T_scr[:, cols] = x1
                hnT_scr[:, cols] = two_ln(x1.astype(F32))[2].astype(BF16)
                go_cps[t].wait()
                goT = io_buf[t].T
                goT_scr[:, cols] = goT
                db2.append(jnp.sum(goT.astype(F32) * _lanes(col_scr[3], TC), axis=0, keepdims=True))
            db2_ref[...] = jnp.concatenate(db2, axis=1).reshape(S).astype(BF16)

            def mlp_chunk(f, slot, n, first):
                for cp in w_cps(f, slot, n):
                    cp.wait()
                w1c = w1_buf.at[slot, pl.ds(0, n)]
                w2c = w2_buf.at[slot, pl.ds(0, n)]
                frows = pl.ds(pl.multiple_of(f * FC, FC), n)
                u = _dot_nt(w1c[...], hnT_scr[...]) + _lanes(b1c_scr[frows, :], D)
                dg = _dot_nt(w2c[...], goT_scr[...]) * gb
                g, dgelu = _gelu_and_grad(u)
                du_b = (dg * dgelu).astype(BF16)
                gg_b = (g * gb).astype(BF16)
                gT = g.astype(BF16).T
                duT = du_b.T
                db1_scr[f, :, 0:n] = jnp.sum(duT.astype(F32), axis=0, keepdims=True)
                for t in range(NTC):
                    cols = pl.ds(t * TC, TC)
                    dw2_buf[slot, 0:n, cols] = _dot(gg_b, goT_scr[:, cols]).astype(BF16)
                    dw1_buf[slot, 0:n, cols] = _dot(du_b, hnT_scr[:, cols]).astype(BF16)
                for t in range(NTC):
                    cols = pl.ds(t * TC, TC)
                    y = _dot(gT, w2c[:, cols])
                    dhn = _dot(duT, w1c[:, cols])
                    if first:
                        y_scr[:, cols] = y
                        dhn_scr[:, cols] = dhn
                    else:
                        y_scr[:, cols] += y
                        dhn_scr[:, cols] += dhn
                for cp in dw_cps(f, slot, n):
                    cp.start()

            mlp_chunk(NFC, NFC & 1, FTAIL, True)

            def mlp_body(i, carry):
                f = NFC - 1 - i
                slot = f & 1

                @pl.when(f > 0)
                def _():
                    for cp in w_cps(f - 1, 1 - slot, FC):
                        cp.start()

                @pl.when(i == 1)
                def _():
                    for cp in dw_cps(NFC, NFC & 1, FTAIL):
                        cp.wait()

                @pl.when(i > 1)
                def _():
                    for cp in dw_cps(f + 2, slot, FC):
                        cp.wait()

                mlp_chunk(f, slot, FC, False)
                return carry

            lax.fori_loop(0, NFC, mlp_body, 0)
            db1 = [db1_scr[f] for f in range(NFC)] + [db1_scr[NFC, :, 0:FTAIL]]
            db1_ref[...] = jnp.concatenate(db1, axis=1).reshape(F).astype(BF16)

            woT_scr[...] = (wo_buf[...].astype(F32) * ga).astype(BF16)
            out_cps = [
                pltpu.make_async_copy(io_buf.at[t], out_hbm.at[pl.ds(t * TC, TC)], sems.at[2 + t])
                for t in range(NTC)
            ]
            for t in range(NTC):
                cols = pl.ds(t * TC, TC)
                x1 = x1T_scr[:, cols].astype(F32)
                go = goT_scr[:, cols].astype(F32)
                y = y_scr[:, cols] + b2[:, t * TC:(t + 1) * TC]
                io_buf[t] = (x1 + _lanes(col_scr[3], TC) * y).astype(BF16).T
                out_cps[t].start()
                xh1, rstd1, hn, rstd2 = two_ln(x1)
                dh2 = _ln_bwd(dhn_scr[:, cols], hn, rstd2)
                parts = (_fold_lanes(dh2), _fold_lanes(dh2 * xh1), _fold_lanes(go * y))
                for i, part in enumerate(parts):
                    if t == 0:
                        part_scr[i] = part
                    else:
                        part_scr[i] += part
                dx1 = (go + _ln_bwd(dh2 * _lanes(col_scr[2], TC), xh1, rstd1)).astype(BF16)
                dx1_scr[:, cols] = dx1
                oT = oT_scr[:, cols]
                gpart = _dot_nt(oT, dx1)
                if t == 0:
                    g_scr[...] = gpart
                else:
                    g_scr[...] += gpart
                doT = _dot(woT_scr[...], dx1)
                for h in range(H):
                    rows = slice(h * DH, (h + 1) * DH)
                    do_b = (doT[rows] * linv_scr[h:h + 1, cols]).astype(BF16)
                    delta_scr[h:h + 1, cols] = jnp.sum(
                        do_b.astype(F32) * oT[rows].astype(F32), axis=0, keepdims=True)
                    oT_scr[rows, cols] = do_b

            gmat = g_scr[...]
            dga = jnp.sum(gmat * wo_buf[...].astype(F32), axis=0, keepdims=True)
            wo_buf[...] = (gmat * ga).astype(BF16)
            dwo_cp = pltpu.make_async_copy(wo_buf, dwo_hbm, sems.at[0])
            dwo_cp.start()
            dmod = jnp.concatenate([dga] + [_col_sum_to_row(part_scr[i]) for i in range(3)], axis=1)
            dcp_scr[...] = _dot_nt(jnp.broadcast_to(dmod.astype(BF16), (16, 4 * D)), wm_buf[...])
            sc_col = _row_to_col(sc.astype(F32))
            wm_buf[...] = (_lanes(sc_col, 4 * D) * dmod).astype(BF16)
            dwm_cp = pltpu.make_async_copy(wm_buf, dwm_hbm.at[:, pl.ds(2 * D, 4 * D)], sems.at[1])
            dwm_cp.start()
            for f in (1, 0):
                for cp in dw_cps(f, f & 1, FC):
                    cp.wait()
            for cp in out_cps:
                cp.wait()
            dwo_cp.wait()
            dwm_cp.wait()

        with jax.named_scope("mid"):
            pl.run_scoped(
                phase_mid,
                pltpu.VMEM((NTC, TC, D), BF16), pltpu.VMEM((D, S), BF16), pltpu.VMEM((D, S), BF16),
                pltpu.VMEM((D, D), BF16), pltpu.VMEM((D, D), BF16), pltpu.VMEM((D, 4 * D), BF16),
                pltpu.VMEM((4, D, 128), F32), pltpu.VMEM((FPAD, 128), F32),
                pltpu.VMEM((2, FC, S), BF16), pltpu.VMEM((2, FC, S), BF16),
                pltpu.VMEM((2, FC, S), BF16), pltpu.VMEM((2, FC, S), BF16),
                pltpu.VMEM((D, S), F32), pltpu.VMEM((D, S), F32),
                pltpu.VMEM((NFC + 1, 1, FC), F32), pltpu.VMEM((D, D), F32), pltpu.VMEM((3, D, 128), F32),
            )

        def phase_bwd(dkT_scr, dvT_scr, pre_scr, wq_buf, wm_buf, dx_buf, g_scr, part_scr):
            wq_cp = pltpu.make_async_copy(wq_hbm, wq_buf, sems.at[0])
            wm_cp = pltpu.make_async_copy(wm_hbm.at[:, pl.ds(0, 2 * D)], wm_buf, sems.at[1])
            wq_cp.start()
            wm_cp.start()
            dkT_scr[...] = jnp.zeros((DH, S), F32)
            dvT_scr[...] = jnp.zeros((DH, S), F32)

            def step(b, slot):
                q, do, delta, m, where, dq, ds = {}, {}, {}, {}, {}, {}, {}
                for u in range(UN):
                    h, rows, cols = qslice(b, u)
                    where[u] = (rows, cols)
                    q[u] = qT_scr[rows, cols]
                    do[u] = oT_scr[rows, cols]
                    delta[u] = jnp.broadcast_to(delta_scr[pl.ds(h, 1), cols], (8, CW))
                    if slot is None:
                        m[u] = jnp.broadcast_to(m_scr[pl.ds(h, 1), cols], (8, CW))

                def probs(u, kt):
                    if slot is None:
                        return pltpu.bitcast(pre_scr[(u * NKT + kt) % 8], BF16)
                    return pltpu.bitcast(p_scr[slot, u, pl.ds(kt * (KT // 2), KT // 2), :], BF16)

                def do_p(u, kt):
                    s = _dot(key_rows(k_scr, kt), q[u]).reshape(KT // 8, 8, CW)
                    p = jnp.exp2(s - m[u][None]).reshape(KT, CW).astype(BF16)
                    pre_scr[(u * NKT + kt) % 8] = pltpu.bitcast(p, U32)

                def do_ds(u, kt):
                    dp = _dot(key_rows(v_scr, kt), do[u]).reshape(KT // 8, 8, CW) - delta[u][None]
                    ds[u, kt] = (probs(u, kt).astype(F32) * dp.reshape(KT, CW)).astype(BF16)

                def do_dv(u, kt):
                    dvT_scr[:, pl.ds(kt * KT, KT)] += _dot_nt(do[u], probs(u, kt))

                def do_dk(u, kt):
                    dkT_scr[:, pl.ds(kt * KT, KT)] += _dot_nt(q[u], ds[u, kt])

                def do_dq(u, kt):
                    t = _dot(key_cols(kT_scr, kt), ds[u, kt])
                    dq[u] = t if kt == 0 else dq[u] + t
                    if kt == NKT - 1:
                        oT_scr[where[u]] = (dq[u] * SCALE).astype(BF16)

                tiles = [(u, kt) for u in range(UN) for kt in range(NKT)]
                if slot is None:
                    plan = ((do_p, 0), (do_dv, LAG), (do_ds, LAG), (do_dk, 2 * LAG), (do_dq, 2 * LAG))
                else:
                    plan = ((do_ds, 0), (do_dv, 0), (do_dk, LAG), (do_dq, LAG))
                for i in range(len(tiles) + 2 * LAG):
                    for fn, lag in plan:
                        if 0 <= i - lag < len(tiles):
                            fn(*tiles[i - lag])

            def stored_body(i, carry):
                n = N_HBM + N_VMEM - 1 - i
                b = jnp.where(n < N_HBM, n, n + N_REC)

                @pl.when(n < N_HBM)
                def _():
                    fill(n).wait()

                step(b, lax.rem(n, N_VMEM))

                @pl.when(n >= N_VMEM)
                def _():
                    fill(n - N_VMEM).start()

                @pl.when(n == N_HBM)
                def _():
                    def rec_body(r, carry):
                        step(N_HBM + r, None)
                        return carry

                    lax.fori_loop(0, N_REC, rec_body, 0)

                return carry

            with jax.named_scope("attn_bwd"):
                lax.fori_loop(0, N_HBM + N_VMEM, stored_body, 0)

            wq_cp.wait()
            wm_cp.wait()
            dkv = jnp.concatenate([dkT_scr[...] * (1.0 / LOG2E), dvT_scr[...]], axis=0).astype(BF16)
            wkv = jnp.concatenate(
                [wkT_ref[...], wvT_ref[...], jnp.zeros((128 - 2 * DH, D), BF16)], axis=0).T[:, 0:2 * DH]
            dx_cps = [
                pltpu.make_async_copy(dx_buf.at[t], dx_hbm.at[pl.ds(t * TC, TC)], sems.at[2 + t])
                for t in range(NTC)
            ]
            dwkv = None
            for t in range(NTC):
                cols = pl.ds(t * TC, TC)
                dqT = oT_scr[:, cols]
                dkv_t = dkv[:, t * TC:(t + 1) * TC]
                dh = _dot(wq_buf[...], dqT) + _dot(wkv, dkv_t)
                xhat, rstd = _ln(xT_scr[:, cols].astype(F32))
                a1 = _lanes(a1_scr[...], TC)
                hT = (xhat * a1 + _lanes(a0_scr[...], TC)).astype(BF16)
                for i, part in enumerate((_fold_lanes(dh), _fold_lanes(dh * xhat))):
                    if t == 0:
                        part_scr[i] = part
                    else:
                        part_scr[i] += part
                dx = dx1_scr[:, cols].astype(F32) + _ln_bwd(dh * a1, xhat, rstd)
                dx_buf[t] = dx.astype(BF16).T
                dx_cps[t].start()
                gpart = _dot_nt(hT, dqT)
                if t == 0:
                    g_scr[...] = gpart
                else:
                    g_scr[...] += gpart
                part = _dot_nt(dkv_t, hT)
                dwkv = part if dwkv is None else dwkv + part

            dmod = jnp.concatenate([_col_sum_to_row(part_scr[i]) for i in range(2)], axis=1)
            dsc = _dot_nt(jnp.broadcast_to(dmod.astype(BF16), (16, 2 * D)), wm_buf[...]) + dcp_scr[...]
            sc_col = _row_to_col(sc.astype(F32))
            wm_buf[...] = (_lanes(sc_col, 2 * D) * dmod).astype(BF16)
            dwm_cp = pltpu.make_async_copy(wm_buf, dwm_hbm.at[:, pl.ds(0, 2 * D)], sems.at[1])
            dwm_cp.start()
            wq_buf[...] = g_scr[...].astype(BF16)
            dwq_cp = pltpu.make_async_copy(wq_buf, dwq_hbm, sems.at[0])
            dwq_cp.start()
            dc_ref[...] = (dsc[0:1] * (sig_c * (1.0 + c * (1.0 - sig_c)))).astype(BF16)
            dwkT_ref[...] = dwkv[0:DH].astype(BF16)
            dwvT_ref[...] = dwkv[DH:2 * DH].astype(BF16)
            for cp in dx_cps:
                cp.wait()
            dwm_cp.wait()
            dwq_cp.wait()

        with jax.named_scope("bwd"):
            pl.run_scoped(
                phase_bwd,
                pltpu.VMEM((DH, S), F32), pltpu.VMEM((DH, S), F32), pltpu.VMEM((8, KT // 2, CW), U32),
                pltpu.VMEM((D, D), BF16), pltpu.VMEM((D, 2 * D), BF16), pltpu.VMEM((NTC, TC, D), BF16),
                pltpu.VMEM((D, D), F32), pltpu.VMEM((2, D, 128), F32),
            )

    pl.run_scoped(phase_rest, pltpu.VMEM((D, S), BF16))


@jax.jit
def pallas_adaLN_cond__grouped_kv_mqa__mixer_token_mlp__prompt_kernel(
    A_x: jax.Array,
    A_wq: jax.Array,
    A_wk: jax.Array,
    A_wv: jax.Array,
    A_wo: jax.Array,
    B_x: jax.Array,
    B_w1: jax.Array,
    B_b1: jax.Array,
    B_w2: jax.Array,
    B_b2: jax.Array,
    c: jax.Array,
    w_mod: jax.Array,
    grad_out: jax.Array,
):
    del B_x
    vmem = pl.BlockSpec(memory_space=pltpu.VMEM)
    hbm = pl.BlockSpec(memory_space=pl.ANY)
    sds = jax.ShapeDtypeStruct
    (dwkT, dwvT, db1, db2, dc, out, dx, dwq, dwo, dw1T, dw2, dwm, _) = pl.pallas_call(
        _kernel,
        in_specs=[vmem] * 5 + [hbm] * 7,
        out_specs=[vmem] * 5 + [hbm] * 8,
        out_shape=[
            sds((DH, D), BF16), sds((DH, D), BF16), sds((F,), BF16), sds((S,), BF16), sds((1, D), BF16),
            sds((S, D), BF16), sds((S, D), BF16), sds((D, D), BF16), sds((D, D), BF16),
            sds((F, S), BF16), sds((F, S), BF16), sds((D, 6 * D), BF16),
            sds((N_HBM, UN, S // 2, CW), U32),
        ],
        scratch_shapes=[
            pltpu.VMEM((N_VMEM, UN, S // 2, CW), U32),
            pltpu.VMEM((D, S), BF16),
            pltpu.VMEM((D, S), BF16),
            pltpu.VMEM((D, S), BF16),
            pltpu.VMEM((S // 2, DH), U32),
            pltpu.VMEM((S // 2, DH), U32),
            pltpu.VMEM((DH // 2, S), U32),
            pltpu.VMEM((DH // 2, S), U32),
            pltpu.VMEM((H, S), F32),
            pltpu.VMEM((H, S), F32),
            pltpu.VMEM((H, S), F32),
            pltpu.VMEM((D, 128), F32),
            pltpu.VMEM((D, 128), F32),
            pltpu.VMEM((16, D), F32),
            pltpu.SemaphoreType.DMA((N_VMEM,)),
            pltpu.SemaphoreType.DMA((14,)),
        ],
        compiler_params=pltpu.CompilerParams(vmem_limit_bytes=127 * 2 ** 20),
    )(c, B_b1, B_b2, A_wk.T, A_wv.T,
      A_x.reshape(S, D), grad_out.reshape(S, D), A_wq, A_wo, B_w1.T, B_w2, w_mod)
    return (out.reshape(1, S, D), dx.reshape(1, S, D), dwq, dwkT.T, dwvT.T, dwo,
            dw1T.T, db1, dw2, db2, dc, dwm)
```

```python
import functools
import math

import jax
import jax.numpy as jnp
from jax import lax
import jax.experimental.pallas as pl
import jax.experimental.pallas.tpu as pltpu

F32 = jnp.float32
BF16 = jnp.bfloat16
U32 = jnp.uint32

S = 2048
D = 512
H = 32
DH = 16
F = 1376
EPS = 1e-5
LOG2E = math.log2(math.e)
SCALE = DH ** -0.5

KT = 128
NKT = S // KT
CW = 512
UN = 2
BQ = CW * UN
NQ = S // BQ
NB = H * NQ
N_VMEM = 30
N_HBM = NB - N_VMEM
FWD_STEPS = 2
FWD_HEAD, FWD_TAIL = 2, 2
MIN_ROW_SUM = 2.0 ** -60
TINY = 2.0 ** -120
BWD_STEPS = 3
PK = 7 * KT // 16

TC = 512
NTC = S // TC
RB = 128
NRB = D // RB
NJ = S // 128
FC = 256
NFC = F // FC
FTAIL = F - NFC * FC
FPAD = -(-F // 128) * 128

WM_ROW = S
W2_ROW, W1_ROW = 0, S
TAIL_ROW = S + F
OUT_ROWS = (TAIL_ROW, F)
STAGE_ROWS = TAIL_ROW + 2 * NTC * FTAIL


def _rows(r):
    return pl.ds(r * RB, RB)


def _packed_rows(r):
    return pl.ds(r * (RB // 2), RB // 2)


NT_DIMS = (((1,), (1,)), ((), ()))


def _dot(a, b):
    return jnp.dot(a, b, preferred_element_type=F32)


def _dot_nt(a, b):
    return lax.dot_general(a, b, NT_DIMS, preferred_element_type=F32)


def _lanes(col, n):
    return jnp.concatenate([col] * (n // 128), axis=1)


def _row_to_col(row):
    n = row.shape[1]
    return jnp.concatenate(
        [jnp.broadcast_to(row[:, j:j + 128], (128, 128)).T for j in range(0, n, 128)], axis=0)


def _col_sum_to_row(part):
    return jnp.sum(part.T, axis=0, keepdims=True)


def _pack(x):
    return pltpu.bitcast(x.astype(BF16), U32)


def _unpack(x):
    return pltpu.bitcast(x, BF16)


TOP_BITS = 0xC000C000


def _squeeze_probs(words):
    last = words[56:64]
    return jnp.concatenate(
        [words[8 * i:8 * i + 8] | ((last << (14 - 2 * i)) & jnp.uint32(TOP_BITS)) for i in range(7)],
        axis=0)


def _expand_probs(words):
    rows, last = [], None
    for i in range(7):
        w = words[8 * i:8 * i + 8]
        top = w & jnp.uint32(TOP_BITS)
        rows.append(w ^ top)
        top = top >> (14 - 2 * i)
        last = top if last is None else last | top
    return jnp.concatenate(rows + [last], axis=0)


def _bf16_pieces(x):
    hi = x.astype(BF16).astype(F32)
    mid = (x - hi).astype(BF16).astype(F32)
    row = lax.broadcasted_iota(jnp.int32, x.shape, 0)
    return jnp.where(row == 0, hi, jnp.where(row == 1, mid, jnp.where(row == 2, x - hi - mid, 0.0)))


def _side_tables(rowsT, ones_ref, turn_ref, kt, sides, order=lambda x: x):
    ones = (lax.broadcasted_iota(jnp.int32, (8, KT), 0) < 3).astype(F32)
    rows = order(jnp.concatenate([rowsT, ones], axis=0).T)
    ones_ref[pl.ds(kt * KT, KT), :] = rows
    shape = (8, rows.shape[1])
    gap = lax.broadcasted_iota(jnp.int32, shape, 1) - lax.broadcasted_iota(jnp.int32, shape, 0)
    for entry, first in sides:
        side = rows[first:first + 8]
        for r in range(8):
            turned = pltpu.roll(side, r + 1, 0) if r < 7 else side
            for half in range(2):
                diagonal = jnp.sum(jnp.where(gap == 8 * half, turned, 0.0), axis=1, keepdims=True)
                turn_ref[entry, 8 * half + r] = jnp.broadcast_to(diagonal, (8, 128))


def _side_product(turn_ref, entry, rhs, acc):
    for r in range(8):
        acc = (pltpu.roll(acc, 1, 0) if r else acc) + _lanes(turn_ref[entry, r], CW) * rhs[0:8]
        acc = acc + _lanes(turn_ref[entry, 8 + r], CW) * rhs[8:16]
    return acc


def _flip_groups(x):
    return jnp.concatenate([x[r:r + 16] for r in reversed(range(0, x.shape[0], 16))], axis=0)


def _sum0(x):
    rows, n = x.shape
    return jnp.sum(jnp.sum(x.reshape(rows // 32, 32, n), axis=0), axis=0, keepdims=True)


class _ColumnSums:
    def __init__(self, count):
        self.acc = [None] * count

    def add(self, *blocks):
        for i, x in enumerate(blocks):
            for r in range(0, x.shape[0], 16):
                self.acc[i] = x[r:r + 16] if self.acc[i] is None else self.acc[i] + x[r:r + 16]

    def rows(self, scale=1.0):
        return [jnp.sum(a, axis=0, keepdims=True) * scale for a in self.acc]


class _Moments:
    def __init__(self):
        self.sums, self.pivot = _ColumnSums(2), None

    def add(self, x):
        if self.pivot is None:
            self.pivot = x[0:1]
        x = x - self.pivot
        self.sums.add(x, x * x)

    def coeffs(self):
        mean, msq = self.sums.rows(1.0 / D)
        rstd = lax.rsqrt(jnp.maximum(msq - mean * mean, 0.0) + EPS)
        return rstd, (mean + self.pivot) * rstd


def _gelu_and_grad(u):
    k0 = math.sqrt(2.0 / math.pi)
    k1 = 0.044715
    u2 = u * u
    t = jnp.tanh(u * (k0 + (k0 * k1) * u2))
    cdf = 0.5 + 0.5 * t
    grad = cdf + (0.5 * u) * (1.0 - t * t) * (k0 + (3.0 * k0 * k1) * u2)
    return u * cdf, grad


def _pipeline(*stages):
    for i in range(NJ * NRB + max(lag for _, lag in stages)):
        for fn, lag in stages:
            if 0 <= i - lag < NJ * NRB:
                fn(*divmod(i - lag, NRB))


def _kernel(
    c_hbm, b1_hbm, b2_hbm, wkT_hbm, wvT_hbm, x_hbm, go_hbm, wq_hbm, wo_hbm, w1T_hbm, w2_hbm, wm_hbm,
    dwkT_hbm, dwvT_hbm, db1_hbm, db2_hbm, dc_hbm,
    out_hbm, dx_hbm, dwq_hbm, dwo_hbm, dw1T_hbm, dw2_hbm, dwm_hbm, p_hbm, q_hbm,
    p_scr, xT_scr, qT_scr, oT_scr, kT_scr, vT_scr, row_scr, mod_scr, dmod_scr, stat_scr,
    c_buf, b1_buf, b2_buf, wkT_buf, wvT_buf, zero_ref, p_sems, sems, small_sems,
):
    zero_ref[0] = 0

    def small_cp(i, src, dst):
        return pltpu.make_async_copy(src, dst, small_sems.at[i])

    def silu_c():
        c = c_buf[...].astype(F32)
        return (c * jax.nn.sigmoid(c)).astype(BF16)

    def qslice(b, u):
        h = lax.shift_right_logical(b, NQ.bit_length() - 1)
        j = b & (NQ - 1)
        cols = pl.ds(pl.multiple_of(j * BQ + u * CW, CW), CW)
        return h, pl.ds(pl.multiple_of(h * (DH // 2), DH // 2), DH // 2), cols

    def tile_rows(i):
        return pl.ds(i * (KT // 2), KT // 2)

    def key_cols(ref, kt):
        return _unpack(ref[:, pl.ds(kt * KT, KT)])

    def spill(n, slot, u):
        return pltpu.make_async_copy(p_scr.at[slot, u], p_hbm.at[n, u], p_sems.at[slot * UN + u])

    def fill(n, slot):
        return pltpu.make_async_copy(p_hbm.at[n], p_scr.at[slot], p_sems.at[slot * UN])

    def q_fill(t):
        cols = pl.ds(pl.multiple_of(t * TC, TC), TC)
        return pltpu.make_async_copy(q_hbm.at[:, cols], qT_scr.at[:, cols], sems.at[18 + t])

    def phase_qkv(wo_cp, wo_buf, woT_buf, prefetches, k_scr, k1_scr, krot_scr, factor_scr,
                  x_buf, wm_buf, wq_buf, wT_scr, col_scr, hT_scr):
        wm_cp = pltpu.make_async_copy(wm_hbm.at[:, pl.ds(0, 2 * D)], wm_buf, sems.at[0])
        wq_cp = pltpu.make_async_copy(wq_hbm, wq_buf, sems.at[1])
        edges = (0, 256, 512, 1024, 2048)
        x_cps = {
            lo: pltpu.make_async_copy(
                x_hbm.at[pl.ds(lo, hi - lo)], x_buf.at[pl.ds(lo, hi - lo)], sems.at[2 + i])
            for i, (lo, hi) in enumerate(zip(edges, edges[1:]))
        }
        small = [
            small_cp(i, *pair) for i, pair in enumerate((
                (c_hbm, c_buf), (wkT_hbm, wkT_buf), (wvT_hbm, wvT_buf),
                (b1_hbm, b1_buf), (b2_hbm, b2_buf)))
        ]
        for cp in [wm_cp, x_cps[0]] + small[0:3]:
            cp.start()
        small[0].wait()
        wq_cp.start()
        wm_cp.wait()
        mod = _dot(jnp.broadcast_to(silu_c(), (16, D)), wm_buf[...])[0:1]
        mod_scr[:, 0:2 * D] = mod
        col_scr[0] = _row_to_col(mod[:, 0:D])
        col_scr[1] = _row_to_col(1.0 + mod[:, D:2 * D])
        sums, coeffs, products, k_norms = {}, {}, {}, []

        def load_tokens(j, r):
            cols = pl.ds(j * 128, 128)
            if r == 0:
                sums[j] = _Moments()
                if j * 128 in x_cps:
                    x_cps[j * 128].wait()
                if j == 0:
                    for cp in list(x_cps.values())[1:] + [wo_cp]:
                        cp.start()
                if j * 128 == edges[-2]:
                    wo_cp.wait()
                    woT_buf[...] = _pack(wo_buf[...].T)
                    for cp in small[3:] + prefetches:
                        cp.start()
            xT = x_buf[cols, _rows(r)].T
            xT_scr[_packed_rows(r), cols] = _pack(xT)
            sums[j].add(xT.astype(F32))
            if r == NRB - 1:
                coeffs[j] = sums[j].coeffs()
                stat_scr[3:4, cols], stat_scr[4:5, cols] = coeffs[j]

        def modulate(j, r):
            cols = pl.ds(j * 128, 128)
            xhat = _unpack(xT_scr[_packed_rows(r), cols]).astype(F32) * coeffs[j][0] - coeffs[j][1]
            hT_scr[_packed_rows(r), cols] = _pack(xhat * col_scr[1, _rows(r)] + col_scr[0, _rows(r)])

        def project(j, r):
            cols = pl.ds(j * 128, 128)
            if j == 0 and r == 0:
                for cp in [wq_cp] + small[1:3]:
                    cp.wait()
                wT_scr[(D + DH) // 2:D // 2 + DH, :] = _pack(wvT_buf[...])
                wT_scr[D // 2:(D + DH) // 2, :] = _pack(wkT_buf[...])
                wT_scr[0:D // 2, :] = _pack(wq_buf[...].T)
            n = RB + 2 * DH if r == NRB - 1 else RB
            products[j, r] = _dot(
                _unpack(wT_scr[pl.ds(r * (RB // 2), n // 2), :]), _unpack(hT_scr[:, cols]))

        def keep(j, r):
            cols, qkv = pl.ds(j * 128, 128), products[j, r]
            q = qkv[0:RB] * (SCALE * LOG2E)
            qT_scr[_packed_rows(r), cols] = _pack(q)
            for i in range(RB // DH):
                h, qh = r * (RB // DH) + i, q[i * DH:(i + 1) * DH]
                row_scr[h:h + 1, cols] = jnp.sum(qh * qh, axis=0, keepdims=True)
            if r == NRB - 1:
                kT_scr[:, cols] = _pack(qkv[RB:RB + DH])
                vT_scr[:, cols] = _pack(qkv[RB + DH:RB + 2 * DH])
                k = qkv[RB:RB + DH]
                k_scr[pl.ds(j * (KT // 2), KT // 2), :] = _pack(_flip_groups(k.T))
                _side_tables(k.astype(BF16).astype(F32), k1_scr, krot_scr, j, [(j, KT - 8)], _flip_groups)
                k_norms.append(jnp.sum(k * k, axis=0, keepdims=True))
                row_scr[0:H, cols] = jnp.sqrt(row_scr[0:H, cols] + TINY)

        _pipeline((project, 2 * NRB), (modulate, NRB), (load_tokens, 0), (keep, 2 * NRB + 1))
        for cp in small[3:]:
            cp.wait()
        k_max = jnp.max(functools.reduce(jnp.maximum, k_norms), axis=1, keepdims=True)
        factor_scr[...] = jnp.broadcast_to(jnp.sqrt(k_max + TINY) * (1.0 + 2.0 ** -6), (8, CW))

    def phase_fwd_mid(stage, wo_buf, woT_buf, col_scr):
        wo_cp = pltpu.make_async_copy(wo_hbm, wo_buf, sems.at[6])
        late = 11 * 128
        halves = (pl.ds(0, late), pl.ds(late, S - late))
        go_cps = [
            pltpu.make_async_copy(go_hbm.at[halves[i]], stage.at[halves[i]], sems.at[16])
            for i in range(2)
        ]
        q_cps = [
            pltpu.make_async_copy(qT_scr.at[:, halves[i]], q_hbm.at[:, halves[i]], sems.at[9])
            for i in range(2)
        ]

        wm_cps = [
            pltpu.make_async_copy(
                wm_hbm.at[:, pl.ds((2 + i) * D, D)], stage.at[pl.ds(WM_ROW + i * D, D)],
                sems.at[8])
            for i in range(4)
        ]

        def phase_attn_fwd(acc_scr, words_scr, cast_scr, l_scr, low_scr, k_scr, k1_scr,
                           krot_scr, factor_scr):
            pl.run_scoped(
                functools.partial(
                    phase_qkv, wo_cp, wo_buf, woT_buf, wm_cps[:3] + go_cps[:1], k_scr, k1_scr,
                    krot_scr, factor_scr),
                pltpu.VMEM((S, D), BF16), pltpu.VMEM((D, 2 * D), BF16),
                pltpu.VMEM((D, D), BF16), pltpu.VMEM((D // 2 + DH, D), U32),
                pltpu.VMEM((2, D, 128), F32), pltpu.VMEM((D // 2, S), U32),
            )
            q_cps[0].start()

            def exact_maxima(i, carry):
                h, rows, cols = qslice(i // UN, i % UN)
                s = _dot(_unpack(k_scr[...]), _unpack(qT_scr[rows, cols]))
                row_scr[pl.ds(h, 1), cols] = jnp.max(s, axis=0, keepdims=True)
                return carry

            def p_times_v(b, u, kt, words, l):
                pv = _dot(key_cols(vT_scr, kt), _unpack(words))
                if kt == 0:
                    acc_scr[0:DH] = pv
                elif kt < NKT - 1:
                    acc_scr[0:DH] += pv
                else:
                    h, rows, cols = qslice(jnp.where(b < 0, b + NB + NQ, b), u)
                    l = jnp.sum(l, axis=0, keepdims=True)
                    low_scr[...] += jnp.where(l >= MIN_ROW_SUM, 0.0, 1.0)
                    row_scr[pl.ds(h, 1), cols] = 1.0 / l
                    oT_scr[rows, cols] = _pack((acc_scr[0:DH] + pv) * (1.0 / l))

            def steps(b, slot, count, offset=None):
                slots = [slot]
                for _ in range(count):
                    slots.append(jnp.where(slots[-1] == N_VMEM - 1, 0, slots[-1] + 1))

                def claim(k, u):
                    @pl.when(b + k >= N_VMEM)
                    def _():
                        spill(b + k - N_VMEM, slots[k], u).wait()

                def send(k, u):
                    @pl.when(b + k < N_HBM)
                    def _():
                        spill(b + k, slots[k], u).start()

                groups = [(k, u) for k in range(count) for u in range(UN)]
                for group in groups if count > 1 else groups[:1]:
                    claim(*group)
                q, m, rhs, l = {}, {}, {}, {}
                for k in range(count):
                    for u in range(UN):
                        h, rows, cols = qslice(b + k, u)
                        q[k, u] = _unpack(qT_scr[rows, cols])
                        m[k, u] = row_scr[pl.ds(h, 1), cols] * factor_scr[...]
                        rhs[k, u] = jnp.concatenate(
                            [q[k, u].astype(F32), _bf16_pieces(-m[k, u])], axis=0)
                tiles = [(k, u, kt) for k in range(count) for u in range(UN) for kt in range(NKT)]
                queue = [
                    (b - 1, UN - 1, NKT - 2 + i, words_scr[tile_rows(i), :], l_scr[...])
                    for i in range(2)
                ]
                for i, (k, u, kt) in enumerate(tiles):
                    if count == 1 and u > 0 and kt == 0:
                        send(k, u - 1)
                        claim(k, u)
                    if offset is None:
                        s = _dot(_unpack(k_scr[tile_rows(kt), :]), q[k, u])
                        s = s - jnp.concatenate([m[k, u]] * (KT // 8), axis=0)
                    elif i < 3:
                        s = _dot(k1_scr[pl.ds(kt * KT, KT), :], rhs[k, u])
                    else:
                        s = _dot(k1_scr[pl.ds(kt * KT, KT - 8), :], rhs[k, u])
                        s = jnp.concatenate(
                            [s, acc_scr[pl.ds(offset + DH + 8 * (i % 4), 8), :]], axis=0)
                    p = jnp.exp2(s)
                    for r in range(0, KT, 8):
                        l[k, u] = l[k, u] + p[r:r + 8] if (k, u) in l else p[r:r + 8]
                    cast_scr[tile_rows(i % 4), :] = _pack(_flip_groups(p))
                    words = cast_scr[tile_rows(i % 4), :]
                    p_scr[slots[k], u, pl.ds(kt * PK, PK), :] = _squeeze_probs(words)
                    p_times_v(*queue.pop(0))
                    queue.append((b + k, u, kt, words, l[k, u]))
                    if offset is not None and 3 <= i + 1 < len(tiles):
                        k, u, kt = tiles[i + 1]
                        acc_scr[pl.ds(offset + DH + 8 * ((i + 1) % 4), 8), :] = (
                            _side_product(krot_scr, kt, rhs[k, u], -m[k, u]))
                for i, entry in enumerate(queue):
                    words_scr[tile_rows(i), :] = entry[3]
                l_scr[...] = queue[-1][4]
                for group in groups if count > 1 else groups[-1:]:
                    send(*group)
                return slots[count]

            def forward(head):
                acc_scr[...] = jnp.zeros(acc_scr.shape, F32)
                words_scr[...] = jnp.zeros(words_scr.shape, U32)
                l_scr[...] = jnp.ones((8, CW), F32)
                low_scr[...] = jnp.zeros((1, CW), F32)

                def ends(end, slot):
                    lo = jnp.where(end == 0, 0, NB - FWD_TAIL)
                    hi = jnp.where(end == 0, head, NB)
                    slot = lax.fori_loop(lo, hi, lambda b, s: steps(b, s, 1), slot)
                    n = jnp.where(end == 0, (NB - FWD_TAIL - head) // FWD_STEPS, 0)

                    def middle(i, s):
                        zero = pl.multiple_of(lax.shift_right_logical(i, 10), 8)
                        return steps(head + i * FWD_STEPS, s, FWD_STEPS, zero)

                    return lax.fori_loop(0, n, middle, slot)

                lax.fori_loop(0, 2, ends, jnp.int32(0))
                for i in range(2):
                    words = words_scr[tile_rows(i), :]
                    p_times_v(jnp.int32(NB - 1), UN - 1, NKT - 2 + i, words, l_scr[...])

            def attempt(i, needed):
                @pl.when(jnp.logical_and(i == 1, needed))
                def _():
                    lax.fori_loop(0, NB * UN, exact_maxima, 0)
                    factor_scr[...] = jnp.ones((8, CW), F32)

                @pl.when(needed)
                def _():
                    forward(jnp.where(i == 0, FWD_HEAD, NB - FWD_TAIL))

                return jnp.max(low_scr[...]) > 0.0

            lax.fori_loop(0, 2, attempt, True)
            for cp in wm_cps[:3] + [go_cps[0], q_cps[0]]:
                cp.wait()
            for cp in (q_cps[1], go_cps[1], wm_cps[3]):
                cp.start()

        pl.run_scoped(
            phase_attn_fwd,
            pltpu.VMEM((DH + 32, CW), F32), pltpu.VMEM((KT, CW), U32), pltpu.VMEM((2 * KT, CW), U32),
            pltpu.VMEM((8, CW), F32), pltpu.VMEM((1, CW), F32), pltpu.VMEM((S // 2, DH), U32),
            pltpu.VMEM((S, DH + 8), F32), pltpu.VMEM((NKT, DH, 8, 128), F32), pltpu.VMEM((8, CW), F32),
        )

        def phase_mid(hnT_scr, gT_scr, duT_scr, h2_scr, b1_scr, db1_scr):
            goT_scr = qT_scr

            def dw_rows(f, k, t, n):
                if n == FTAIL:
                    return pl.ds(TAIL_ROW + (k * NTC + t) * n, n)
                return pl.ds(pl.multiple_of((f & 1) * S + (k * NTC + t) * n, n), n)

            def dw_cps(f, n):
                rows = pl.ds(pl.multiple_of(f * FC, FC), n)
                return [
                    pltpu.make_async_copy(
                        stage.at[dw_rows(f, k, t, n)], dst.at[rows, pl.ds(t * TC, TC)],
                        sems.at[12 if n == FTAIL else 10 + (f & 1)])
                    for k, dst in enumerate((dw1T_hbm, dw2_hbm)) for t in range(NTC)
                ]

            w1_col, w2_col = (stage.at[pl.ds(row, F)] for row in (W1_ROW, W2_ROW))

            def wcol_cp(k, t):
                src, dst = ((w1T_hbm, w1_col), (w2_hbm, w2_col))[k]
                return pltpu.make_async_copy(
                    src.at[:, pl.ds(pl.multiple_of(t * TC, TC), TC)], dst, sems.at[3 + k])

            def hidden_pass(w1_buf, w2_buf):
                def w_cps(f, n):
                    rows = pl.ds(pl.multiple_of(f * FC, FC), n)
                    return (
                        pltpu.make_async_copy(w1T_hbm.at[rows], w1_buf.at[pl.ds(0, n)], sems.at[6]),
                        pltpu.make_async_copy(w2_hbm.at[rows], w2_buf.at[pl.ds(0, n)], sems.at[7]),
                    )

                for cp in w_cps(0, FC):
                    cp.start()
                b1 = b1_buf[...].astype(F32).reshape(1, F)
                b1 = jnp.concatenate([b1, jnp.zeros((1, (NFC + 1) * FC - F), F32)], axis=1)
                for f in range(NFC + 1):
                    b1_scr[f] = b1[:, f * FC:(f + 1) * FC]

                sums1, sums2, co1, co2 = {}, {}, {}, {}

                def modulation(i):
                    sc = jnp.broadcast_to(silu_c(), (16, D))
                    mod = _dot(sc, stage[pl.ds(WM_ROW + i * D, D), :])[0:1]
                    mod_scr[:, (2 + i) * D:(3 + i) * D] = mod
                    col_scr[i] = _row_to_col(1.0 + mod if i == 2 else mod)

                def residual(j, r):
                    cols, rows = pl.ds(j * 128, 128), _packed_rows(r)
                    if r == 0:
                        sums1[j] = _Moments()
                    if j == 0 and r < 3:
                        modulation(r)
                    a = _dot(_unpack(woT_buf[rows, :]), _unpack(oT_scr[0:D // 2, cols]))
                    x1 = _unpack(xT_scr[rows, cols]).astype(F32) + col_scr[0, _rows(r)] * a
                    xT_scr[rows, cols] = _pack(x1)
                    sums1[j].add(x1)
                    if r == NRB - 1:
                        co1[j] = sums1[j].coeffs()
                        stat_scr[0:1, cols], stat_scr[1:2, cols] = co1[j]

                def norm1(j, r):
                    cols = pl.ds(j * 128, 128)
                    if r == 0:
                        sums2[j] = _Moments()
                    xh1 = _unpack(xT_scr[_packed_rows(r), cols]).astype(F32) * co1[j][0] - co1[j][1]
                    h2 = xh1 * col_scr[2, _rows(r)] + col_scr[1, _rows(r)]
                    h2_scr[j % 2, _rows(r)] = h2
                    sums2[j].add(h2)
                    if r == NRB - 1:
                        co2[j] = sums2[j].coeffs()
                        stat_scr[2:3, cols] = co2[j][0]

                def norm2(j, r):
                    cols = pl.ds(j * 128, 128)
                    if j * 128 == late and r == 0:
                        for cp in (q_cps[1], go_cps[1], wm_cps[3]):
                            cp.wait()
                    hn = h2_scr[j % 2, _rows(r)] * co2[j][0] - co2[j][1]
                    hnT_scr[_packed_rows(r), cols] = _pack(hn)
                    go = stage[cols, _rows(r)]
                    goT_scr[_packed_rows(r), cols] = _pack(go.T)

                _pipeline((residual, 0), (norm2, 2 * NRB), (norm1, NRB))
                modulation(3)

                def chunk(f, n, midway):
                    for cp in w_cps(f, n):
                        cp.wait()
                    gb = mod_scr[:, 5 * D:6 * D]
                    b1_col = _row_to_col(b1_scr[f])[0:n]
                    u = _dot_nt(w1_buf[0:n], _unpack(hnT_scr[...])) + _lanes(b1_col, D)
                    dg = _dot_nt(w2_buf[0:n], _unpack(goT_scr[...])) * gb
                    g, dgelu = _gelu_and_grad(u)
                    gg_b = (g * gb).astype(BF16)
                    du_b = (dg * dgelu).astype(BF16)
                    fcols = pl.ds(pl.multiple_of(f * FC, FC), n)
                    gT_scr[:, fcols] = _pack(g.astype(BF16).T)
                    duT = du_b.T
                    duT_scr[:, fcols] = _pack(duT)
                    db1_scr[f, :, 0:n] = _sum0(duT.astype(F32))
                    midway()
                    for k, lhs, rhs in ((1, gg_b, goT_scr), (0, du_b, hnT_scr)):
                        for t in range(NTC):
                            dw = _dot(lhs, _unpack(rhs[:, pl.ds(t * TC, TC)]))
                            stage[dw_rows(f, k, t, n), :] = dw.astype(BF16)

                def body(f, carry):
                    def midway():
                        @pl.when(f + 1 < NFC)
                        def _():
                            for cp in w_cps(f + 1, FC):
                                cp.start()

                        @pl.when(f + 1 == NFC)
                        def _():
                            for cp in w_cps(NFC, FTAIL):
                                cp.start()

                        @pl.when(f >= 1)
                        def _():
                            for cp in dw_cps(f - 1, FC):
                                cp.wait()

                        @pl.when(f + 1 == NFC)
                        def _():
                            wcol_cp(0, NTC - 1).start()

                    chunk(f, FC, midway)
                    for cp in dw_cps(f, FC):
                        cp.start()
                    return carry

                lax.fori_loop(0, NFC, body, 0)
                chunk(NFC, FTAIL, lambda: None)
                for cp in dw_cps(NFC - 1, FC):
                    cp.wait()
                wcol_cp(1, NTC - 1).start()
                for cp in dw_cps(NFC, FTAIL):
                    cp.start()

            pl.run_scoped(
                hidden_pass, pltpu.VMEM((FC, S), BF16), pltpu.VMEM((FC, S), BF16))

            def token_pass(b2_scr, db2_scr, g_scr, part_scr):
                da_scr = woT_buf
                b2 = b2_buf[...].astype(F32).reshape(1, S)
                for t in range(NTC):
                    b2_scr[t] = b2[:, t * TC:(t + 1) * TC]

                def out_buf(t):
                    row = jnp.where(t & 1 == 0, OUT_ROWS[0], OUT_ROWS[1])
                    return stage.at[pl.ds(pl.multiple_of(row, 32), TC)]

                def out_cp(t):
                    rows = pl.ds(pl.multiple_of(t * TC, TC), TC)
                    return pltpu.make_async_copy(out_buf(t), out_hbm.at[rows], sems.at[14 + (t & 1)])

                dwo_cp = pltpu.make_async_copy(w2_col.at[pl.ds(0, D)], dwo_hbm, sems.at[0])
                planes = ((col_scr, 1), (h2_scr, 0), (h2_scr, 1), (part_scr, 3))

                def put_e(rows, x):
                    for i, (ref, k) in enumerate(planes):
                        ref[k, rows] = x[:, i * 128:(i + 1) * 128]

                def get_e(rows):
                    return jnp.concatenate([ref[k, rows] for ref, k in planes], axis=1)

                def chunk(step, carry):
                    t = NTC - 1 - step
                    cols = pl.ds(pl.multiple_of(t * TC, TC), TC)
                    wcol_cp(0, t).wait()
                    rstd1, shift1, rstd2 = (stat_scr[i:i + 1, cols] for i in range(3))
                    sub = 32

                    def blocks(r):
                        for i in range(r * RB, (r + 1) * RB, sub):
                            yield i - r * RB, pl.ds(i, sub), pl.ds(i // 2, sub // 2)

                    def load(ref, prow):
                        return _unpack(ref[prow, cols]).astype(F32)

                    def fold(i, rows, x):
                        x = (x[:, 0:128] + x[:, 128:256]) + (x[:, 256:384] + x[:, 384:512])
                        part_scr[i, rows] = jnp.where(step > 0, part_scr[i, rows], 0.0) + x

                    sums = _ColumnSums(2)
                    for r in range(NRB):
                        dhn = _dot(_unpack(duT_scr[_packed_rows(r), 0:F]), w1_col[...])
                        for i, rows, prow in blocks(r):
                            put_e(rows, dhn[i:i + sub])
                            sums.add(dhn[i:i + sub], dhn[i:i + sub] * load(hnT_scr, prow))
                    c0, c1 = (x * rstd2 for x in sums.rows(1.0 / D))

                    @pl.when(t > 0)
                    def _():
                        wcol_cp(0, t - 1).start()

                    @pl.when(step == 1)
                    def _():
                        for cp in dw_cps(NFC, FTAIL):
                            cp.wait()

                    @pl.when(step >= 2)
                    def _():
                        out_cp(t + 2).wait()

                    wcol_cp(1, t).wait()
                    sums, db2 = _ColumnSums(2), _ColumnSums(1)
                    for r in range(NRB):
                        y = _dot(_unpack(gT_scr[_packed_rows(r), 0:F]), w2_col[...])
                        out = []
                        for i, rows, prow in blocks(r):
                            yi = y[i:i + sub] + b2_scr[t]
                            go, gb = load(goT_scr, prow), _lanes(col_scr[3, rows], TC)
                            fold(2, rows, go * yi)
                            db2.add(go * gb)
                            out.append(load(xT_scr, prow) + gb * yi)
                        out_buf(t)[:, _rows(r)] = jnp.concatenate(out, axis=0).astype(BF16).T
                        todo = [blk for rr in range(NRB) for blk in blocks(rr)]
                        if r < NRB - 1:
                            todo = todo[r * len(todo) // (NRB - 1):(r + 1) * len(todo) // (NRB - 1)]
                        else:
                            c0, c1 = (x * rstd1 for x in sums.rows(1.0 / D))
                        for _, rows, prow in todo:
                            xh1 = load(xT_scr, prow) * rstd1 - shift1
                            if r < NRB - 1:
                                dh2 = get_e(rows) * rstd2 - c0 - load(hnT_scr, prow) * c1
                                fold(0, rows, dh2)
                                fold(1, rows, dh2 * xh1)
                                e = dh2 * _lanes(col_scr[2, rows], TC)
                                put_e(rows, e)
                                sums.add(e, e * xh1)
                            else:
                                dx1 = load(goT_scr, prow) + (get_e(rows) * rstd1 - c0 - xh1 * c1)
                                hnT_scr[prow, cols] = _pack(dx1)
                    db2_scr[t] = db2.rows()[0]
                    dga = _ColumnSums(1)
                    for r in range(NRB):
                        prow = _packed_rows(r)
                        o = _unpack(oT_scr[prow, cols])
                        g = jnp.where(step > 0, g_scr[_rows(r), :], 0.0)
                        g = g + _dot_nt(o, _unpack(hnT_scr[:, cols]))
                        g_scr[_rows(r), :] = g
                        if r == 0:
                            out_cp(t).start()
                        xT_scr[prow, cols] = hnT_scr[prow, cols]
                        da_scr[prow, :] = _pack(load(hnT_scr, prow) * _lanes(col_scr[0, _rows(r)], TC))
                        if r < 3:
                            dmod_scr[:, (3 + r) * D:(4 + r) * D] = _col_sum_to_row(part_scr[r])
                        else:
                            db1 = [db1_scr[f] for f in range(NFC)] + [db1_scr[NFC, :, 0:FTAIL]]
                            b1_buf[...] = jnp.concatenate(db1, axis=1).reshape(F).astype(BF16)
                        dga.add(g * wo_buf[_rows(r), :].astype(F32))
                        w2_col[_rows(r), :] = (g * mod_scr[:, 2 * D:3 * D]).astype(BF16)
                    dmod_scr[:, 2 * D:3 * D] = dga.rows()[0]

                    @pl.when(t > 0)
                    def _():
                        wcol_cp(1, t - 1).start()

                    @pl.when(t == 0)
                    def _():
                        dwo_cp.start()

                    q_fill(t).start()

                    @pl.when(zero_ref[0] == 0)
                    def _():
                        for r in range(NRB):
                            doT = _dot(wo_buf[_rows(r), :], _unpack(da_scr[...]))
                            for i in range(RB // DH):
                                h = r * (RB // DH) + i
                                rows = pl.ds(h * DH // 2, DH // 2)
                                do = doT[i * DH:(i + 1) * DH] * row_scr[h:h + 1, cols]
                                row_scr[h:h + 1, cols] = jnp.sum(
                                    do * _unpack(oT_scr[rows, cols]).astype(F32), axis=0, keepdims=True)
                                oT_scr[rows, cols] = _pack(do)

                    return carry

                lax.fori_loop(0, NTC, chunk, 0)
                db2 = jnp.concatenate([db2_scr[t] for t in range(NTC)], axis=1)
                b2_buf[...] = db2.reshape(S).astype(BF16)
                small_cp(3, b1_buf, db1_hbm).start()
                small_cp(4, b2_buf, db2_hbm).start()
                out_cp(jnp.int32(1)).wait()
                out_cp(jnp.int32(0)).wait()
                dwo_cp.wait()

            pl.run_scoped(
                token_pass,
                pltpu.VMEM((NTC, 1, TC), F32), pltpu.VMEM((NTC, 1, TC), F32),
                pltpu.VMEM((D, D), F32), pltpu.VMEM((4, D, 128), F32),
            )

        pl.run_scoped(
            phase_mid,
            pltpu.VMEM((D // 2, S), U32),
            pltpu.VMEM((D // 2, FPAD), U32), pltpu.VMEM((D // 2, FPAD), U32),
            pltpu.VMEM((2, D, 128), F32),
            pltpu.VMEM((NFC + 1, 1, FC), F32), pltpu.VMEM((NFC + 1, 1, FC), F32),
        )

    pl.run_scoped(
        phase_fwd_mid,
        pltpu.VMEM((STAGE_ROWS, D), BF16), pltpu.VMEM((D, D), BF16), pltpu.VMEM((D // 2, D), U32),
        pltpu.VMEM((4, D, 128), F32),
    )

    def phase_bwd(dkT_scr, dvT_scr, ds_scr, dq_scr, x_buf, wq_buf, wm_buf, dwm_buf,
                  v1_scr, vrot_scr, pw_scr, w_scr, col_scr, part_scr):
        hT_scr, dwq_buf = qT_scr, wq_buf
        wq_cp = pltpu.make_async_copy(wq_hbm, wq_buf, sems.at[0])
        wm_cps = {
            r: pltpu.make_async_copy(wm_hbm.at[:, cols], wm_buf.at[:, cols], sems.at[14 + r])
            for r, cols in ((1, pl.ds(0, 4 * D)), (3, pl.ds(4 * D, 2 * D)))
        }
        split = NJ // 2 + 1
        x_cps = {
            lo: pltpu.make_async_copy(
                x_hbm.at[pl.ds(lo * 128, n * 128)], x_buf.at[pl.ds(lo * 128, n * 128)], sems.at[sem])
            for lo, n, sem in ((0, split, 2), (split, NJ - split, 3))
        }
        dkT_scr[...] = jnp.zeros((DH, S), F32)
        dvT_scr[0:DH] = jnp.zeros((DH, S), F32)
        for ref in (ds_scr, pw_scr, dq_scr):
            ref[...] = jnp.zeros(ref.shape, ref.dtype)
        for t in range(1, NTC):
            q_fill(t).wait()

        def value_tables(kt):
            sides = [(kt, 0)] + [(NKT + kt // 2, KT - 8)] * (kt % 2)
            _side_tables(key_cols(vT_scr, kt).astype(F32), v1_scr, vrot_scr, kt, sides)

        value_tables(0)
        value_tables(1)

        def steps(b, slots, offset=None):
            q, do, delta, rhs = {}, {}, {}, {}

            def operands(k):
                for u in range(UN):
                    h, rows, cols = qslice(jnp.minimum(b - k, NB - 1), u)
                    q[k, u], do[k, u] = _unpack(qT_scr[rows, cols]), _unpack(oT_scr[rows, cols])
                    if k >= 0:
                        delta[k, u] = jnp.broadcast_to(row_scr[pl.ds(h, 1), cols], (8, CW))
                        rhs[k, u] = jnp.concatenate(
                            [do[k, u].astype(F32), _bf16_pieces(-delta[k, u])], axis=0)

            for k in range(-1, min(len(slots), 1)):
                operands(k)

            def side_rows(i):
                return pl.ds(offset + DH + 8 * i, 8), pl.ds(0, CW)

            def consume(k, u, kt, p, ds):
                dvT_scr[0:DH, pl.ds(kt * KT, KT)] += _dot_nt(do[k, u], p)
                dkT_scr[:, pl.ds(kt * KT, KT)] += _dot_nt(q[k, u], ds)
                dq, rows = _dot(key_cols(kT_scr, kt), ds), pl.ds(u * DH, DH)
                if kt == 0:
                    dq_scr[rows, :] = dq
                elif kt < NKT - 1:
                    dq_scr[rows, :] += dq
                else:
                    oT_scr[qslice(b - k, u)[1:]] = _pack((dq_scr[rows, :] + dq) * SCALE)

            tiles = [(k, u, kt) for k in range(len(slots)) for kt in range(NKT) for u in range(UN)]
            queue = [
                (-1, u, NKT - 1, _unpack(pw_scr[tile_rows(u), :]), _unpack(ds_scr[tile_rows(u), :]))
                for u in range(UN)
            ]
            for i, (k, u, kt) in enumerate(tiles):
                words = _expand_probs(p_scr[slots[k], u, pl.ds(kt * PK, PK), :])
                if offset is None or i == 0:
                    dp = _dot(v1_scr[pl.ds(kt * KT, KT), :], rhs[k, u])
                elif i % 4 < 3:
                    dp = _dot(v1_scr[pl.ds(kt * KT + 8, KT - 8), :], rhs[k, u])
                    dp = jnp.concatenate([dvT_scr[side_rows(i % 4)], dp], axis=0)
                else:
                    dp = _dot(v1_scr[pl.ds(kt * KT + 8, KT - 16), :], rhs[k, u])
                    dp = jnp.concatenate([dvT_scr[side_rows(3)], dp, dvT_scr[side_rows(4)]], axis=0)
                ds = _unpack(words).astype(F32) * dp
                if i < len(tiles) - UN:
                    queue.append((k, u, kt, _unpack(words), ds.astype(BF16)))
                else:
                    pw_scr[tile_rows(u), :], ds_scr[tile_rows(u), :] = words, _pack(ds)
                consume(*queue.pop(0))
                if offset is None:
                    if u == 0 and kt + 2 < NKT:
                        value_tables(kt + 2)
                    if u == 1 and kt < 3:
                        col_scr[kt] = _row_to_col(
                            (mod_scr[:, 0:D], 1.0 + mod_scr[:, D:2 * D], silu_c().astype(F32))[kt])
                elif i + 1 < len(tiles):
                    k, u, kt = tiles[i + 1]
                    if (k, u) not in rhs:
                        operands(k)
                    dvT_scr[side_rows((i + 1) % 4)] = _side_product(
                        vrot_scr, kt, rhs[k, u], -delta[k, u])
                    if (i + 1) % 4 == 3:
                        dvT_scr[side_rows(4)] = _side_product(
                            vrot_scr, NKT + kt // 2, rhs[k, u], -delta[k, u])
            for entry in queue:
                consume(*entry)

        def body(i, slot):
            b = NB - 1 - peeled - i * BWD_STEPS
            slots = [slot]
            for _ in range(2 * BWD_STEPS - 1):
                slots.append(jnp.where(slots[-1] == 0, N_VMEM - 1, slots[-1] - 1))
            piece = jnp.minimum(i, 15)
            rows = pl.ds(pl.multiple_of((piece & 1) * (D // 2), D // 2), D // 2)
            cols = pl.ds(pl.multiple_of(2 * D + lax.shift_right_logical(piece, 1) * 256, 256), 256)
            dwm_buf[rows, cols] = (_lanes(col_scr[2, rows], 256) * dmod_scr[:, cols]).astype(BF16)
            steps(b, slots[:BWD_STEPS], pl.multiple_of(lax.shift_right_logical(i, 10), 8))
            for k in range(BWD_STEPS):
                @pl.when(b - k >= N_VMEM)
                def _():
                    fill(b - k - N_VMEM, slots[k]).start()

            for k in range(BWD_STEPS, 2 * BWD_STEPS):
                @pl.when(jnp.logical_and(b - k < N_HBM, b - k >= 0))
                def _():
                    fill(b - k, slots[k]).wait()

            return slots[BWD_STEPS]

        peeled = 1
        assert (NB - peeled) % BWD_STEPS == 0
        for cp in [wq_cp, *x_cps.values(), *wm_cps.values()]:
            cp.start()
        steps(NB - 1, [(NB - 1) % N_VMEM])
        fill(NB - 1 - N_VMEM, (NB - 1) % N_VMEM).start()
        q_fill(0).wait()
        lax.fori_loop(0, (NB - peeled) // BWD_STEPS, body, jnp.int32((NB - 1 - peeled) % N_VMEM))
        steps(-1, [])

        wq_cp.wait()
        x_cps[0].wait()
        dkv = jnp.concatenate([dkT_scr[...] * (1.0 / LOG2E), dvT_scr[0:DH]], axis=0).astype(BF16)
        wkv = jnp.concatenate(
            [wkT_buf[...], wvT_buf[...], jnp.zeros((128 - 2 * DH, D), BF16)], axis=0).T[:, 0:2 * DH]
        w_scr[...] = _pack(wq_buf[...])
        dx_cps = [
            pltpu.make_async_copy(x_buf.at[rows], dx_hbm.at[rows], sems.at[18 + i])
            for i, rows in enumerate((pl.ds(0, S // 2), pl.ds(S // 2, S // 2)))
        ]
        out_cps = [
            pltpu.make_async_copy(dwm_buf.at[:, cols], dwm_hbm.at[:, cols], sems.at[6 + i])
            for i, cols in enumerate((pl.ds(2 * D, 4 * D), pl.ds(0, 2 * D)))
        ]
        sums, coeffs = {}, {}

        def put_dwm(i):
            rows, cols = pl.ds(i % 8 * (D // 8), D // 8), pl.ds(i // 8 * 256, 256)
            dwm_buf[rows, cols] = (_lanes(col_scr[2, rows], 256) * dmod_scr[:, cols]).astype(BF16)

        def grad_h(j, r):
            cols, rows = pl.ds(j * 128, 128), _rows(r)
            if r == 0:
                sums[j] = _ColumnSums(2)
                if j == split:
                    dx_cps[0].start()
                    out_cps[0].start()
                    x_cps[split].wait()
            dh = (_dot(_unpack(w_scr[_packed_rows(r), :]), _unpack(oT_scr[0:D // 2, cols]))
                  + _dot(wkv[r * RB:(r + 1) * RB], dkv[:, j * 128:(j + 1) * 128]))
            x = x_buf[cols, rows].T.astype(F32)
            xhat = x * stat_scr[3:4, cols] - stat_scr[4:5, cols]
            hT_scr[_packed_rows(r), cols] = _pack(xhat * col_scr[1, rows] + col_scr[0, rows])
            if j == 0:
                part_scr[0, rows] = dh
                part_scr[1, rows] = dh * xhat
            else:
                part_scr[0, rows] += dh
                part_scr[1, rows] += dh * xhat
            e = dh * col_scr[1, rows]
            vrot_scr[j % 2 * NRB + r] = e.reshape(RB // 8, 8, 128)
            vrot_scr[(2 + j % 2) * NRB + r] = xhat.reshape(RB // 8, 8, 128)
            sums[j].add(e, e * xhat)
            if r == NRB - 1:
                coeffs[j] = [x * stat_scr[3:4, cols] for x in sums[j].rows(1.0 / D)]

        def grad_x(j, r):
            cols, rows = pl.ds(j * 128, 128), _rows(r)
            e, xhat = (vrot_scr[(k + j % 2) * NRB + r].reshape(RB, 128) for k in (0, 2))
            dx = e * stat_scr[3:4, cols] - coeffs[j][0] - xhat * coeffs[j][1]
            dx = dx + _unpack(xT_scr[_packed_rows(r), cols]).astype(F32)
            x_buf[cols, rows] = dx.astype(BF16).T

        _pipeline((grad_h, 0), (grad_x, NRB))
        dx_cps[1].start()
        for i in range(2):
            dmod_scr[:, i * D:(i + 1) * D] = _col_sum_to_row(part_scr[i])
        dwkv = dsc = None
        for r in range(NRB):
            acc = None
            if r in wm_cps:
                wm_cps[r].wait()
            for j in range(NJ):
                cols = pl.ds(j * 128, 128)
                part = _dot_nt(_unpack(hT_scr[_packed_rows(r), cols]), _unpack(oT_scr[0:D // 2, cols]))
                acc = part if acc is None else acc + part
                if r == 0:
                    part = _dot_nt(dkv[:, j * 128:(j + 1) * 128], _unpack(hT_scr[:, cols]))
                    dwkv = part if dwkv is None else dwkv + part
                elif j < 2 * D // 128:
                    cols = pl.ds((r - 1) * 2 * D + j * 128, 128)
                    dmod = jnp.broadcast_to(dmod_scr[:, cols].astype(BF16), (16, 128))
                    part = _dot_nt(dmod, wm_buf[:, cols])
                    dsc = part if dsc is None else dsc + part
                if r == 0:
                    put_dwm(2 * j)
                    put_dwm(2 * j + 1)
            dwq_buf[_rows(r), :] = acc.astype(BF16)
            out_cps.append(
                pltpu.make_async_copy(dwq_buf.at[_rows(r)], dwq_hbm.at[_rows(r)], sems.at[10 + r]))
            out_cps[-1].start()
            if r == 0:
                out_cps[1].start()
                wkT_buf[...] = dwkv[0:DH].astype(BF16)
                wvT_buf[...] = dwkv[DH:2 * DH].astype(BF16)
                out_cps += [small_cp(1, wkT_buf, dwkT_hbm), small_cp(2, wvT_buf, dwvT_hbm)]
                for cp in out_cps[-2:]:
                    cp.start()
        c = c_buf[...].astype(F32)
        sig = jax.nn.sigmoid(c)
        c_buf[...] = (dsc[0:1] * (sig * (1.0 + c * (1.0 - sig)))).astype(BF16)
        out_cps.append(small_cp(0, c_buf, dc_hbm))
        out_cps[-1].start()
        for cp in dx_cps + out_cps + [small_cp(3, b1_buf, db1_hbm), small_cp(4, b2_buf, db2_hbm)]:
            cp.wait()

    pl.run_scoped(
        phase_bwd,
        pltpu.VMEM((DH, S), F32), pltpu.VMEM((DH + 40, S), F32),
        pltpu.VMEM((UN * KT // 2, CW), U32),
        pltpu.VMEM((UN * DH, CW), F32), pltpu.VMEM((S, D), BF16),
        pltpu.VMEM((D, D), BF16), pltpu.VMEM((D, 6 * D), BF16), pltpu.VMEM((D, 6 * D), BF16),
        pltpu.VMEM((S, DH + 8), F32), pltpu.VMEM((NKT + NKT // 2, DH, 8, 128), F32),
        pltpu.VMEM((UN * KT // 2, CW), U32), pltpu.VMEM((D // 2, D), U32),
        pltpu.VMEM((3, D, 128), F32), pltpu.VMEM((2, D, 128), F32),
    )


@jax.jit
def pallas_adaLN_cond__grouped_kv_mqa__mixer_token_mlp__prompt_kernel(
    A_x: jax.Array,
    A_wq: jax.Array,
    A_wk: jax.Array,
    A_wv: jax.Array,
    A_wo: jax.Array,
    B_x: jax.Array,
    B_w1: jax.Array,
    B_b1: jax.Array,
    B_w2: jax.Array,
    B_b2: jax.Array,
    c: jax.Array,
    w_mod: jax.Array,
    grad_out: jax.Array,
):
    del B_x
    hbm = pl.BlockSpec(memory_space=pl.ANY)
    sds = jax.ShapeDtypeStruct
    (dwkT, dwvT, db1, db2, dc, out, dx, dwq, dwo, dw1T, dw2, dwm, _, _) = pl.pallas_call(
        _kernel,
        in_specs=[hbm] * 12,
        out_specs=[hbm] * 14,
        out_shape=[
            sds((DH, D), BF16), sds((DH, D), BF16), sds((F,), BF16), sds((S,), BF16),
            sds((1, D), BF16),
            sds((S, D), BF16), sds((S, D), BF16), sds((D, D), BF16), sds((D, D), BF16),
            sds((F, S), BF16), sds((F, S), BF16), sds((D, 6 * D), BF16),
            sds((N_HBM, UN, NKT * PK, CW), U32), sds((D // 2, S), U32),
        ],
        scratch_shapes=[
            pltpu.VMEM((N_VMEM, UN, NKT * PK, CW), U32),
            pltpu.VMEM((D // 2, S), U32),
            pltpu.VMEM((D // 2, S), U32),
            pltpu.VMEM(((D + DH) // 2, S), U32),
            pltpu.VMEM((DH // 2, S), U32),
            pltpu.VMEM((DH // 2, S), U32),
            pltpu.VMEM((H + 8, S), F32),
            pltpu.VMEM((1, 6 * D), F32),
            pltpu.VMEM((1, 6 * D), F32),
            pltpu.VMEM((8, S), F32),
            pltpu.VMEM((1, D), BF16),
            pltpu.VMEM((F,), BF16),
            pltpu.VMEM((S,), BF16),
            pltpu.VMEM((DH, D), BF16),
            pltpu.VMEM((DH, D), BF16),
            pltpu.SMEM((1,), jnp.int32),
            pltpu.SemaphoreType.DMA((N_VMEM * UN,)),
            pltpu.SemaphoreType.DMA((22,)),
            pltpu.SemaphoreType.DMA((5,)),
        ],
        compiler_params=pltpu.CompilerParams(vmem_limit_bytes=128 * 2 ** 20),
    )(c, B_b1, B_b2, A_wk.T, A_wv.T,
      A_x.reshape(S, D), grad_out.reshape(S, D), A_wq, A_wo, B_w1.T, B_w2, w_mod)
    return (out.reshape(1, S, D), dx.reshape(1, S, D), dwq, dwkT.T, dwvT.T, dwo,
            dw1T.T, db1, dw2, db2, dc, dwm)
```
